```python
import os as _os
_os.environ.setdefault('JAX_PLATFORMS', 'cpu')
import jax
import jax.numpy as jnp

def _softmax(x, axis=-1):
    return jax.nn.softmax(x, axis=axis)

def _gelu(x):
    return jax.nn.gelu(x, approximate=True)

def _silu(x):
    return jax.nn.silu(x)

def _sigmoid(x):
    return jax.nn.sigmoid(x)

def _layernorm(x, axis=-1, eps=1e-05):
    m = jnp.mean(x, axis=axis, keepdims=True)
    v = jnp.var(x, axis=axis, keepdims=True)
    return (x - m) / jnp.sqrt(v + eps)

def _scatter_add(tgt, idx, src, axis=0):
    return tgt.at[idx].add(src)

def _segment_sum(src, seg, n):
    return jax.ops.segment_sum(src, seg, n)

class _Rng:

    def __init__(self, key):
        self._k = key

    def _next(self):
        self._k, sub = jax.random.split(self._k)
        return sub

    def normal(self, shape):
        return jax.random.normal(self._next(), shape, dtype=jnp.bfloat16)

    def randint(self, lo, hi, shape):
        return jax.random.randint(self._next(), shape, lo, hi, dtype=jnp.int32)

    def uniform(self, shape, lo=0.0, hi=1.0):
        return jax.random.uniform(self._next(), shape, jnp.bfloat16, lo, hi)

    def permutation(self, n):
        return jax.random.permutation(self._next(), n)
kernel_name = 'sequential_preLN__linear_attn_block__mixer_gmlp__prompt'

def setup_inputs():
    _rng = _Rng(jax.random.key(int.from_bytes(__import__("os").urandom(4), "little")))
    _w = lambda a: (lambda t: t.astype(jnp.bfloat16) if jnp.issubdtype(t.dtype, jnp.floating) else t)(jnp.asarray(a))

    def _A_setup():
        B, S, D = (1, 2048, 512)
        return {'x': _w((lambda *s: _rng.normal(s) * 0.05)(B, S, D)), 'wqkv': _w((lambda *s: _rng.normal(s) * 0.05)(D, 3 * D)), 'wo': _w((lambda *s: _rng.normal(s) * 0.05)(D, D))}
    _A_in = _A_setup()

    def _B_setup():
        B, S, D, F = (1, 2048, 512, 1792)
        Fh = F // 2
        return {'x': _w((lambda *s: _rng.normal(s) * 0.05)(B, S, D)), 'w_in': _w((lambda *s: _rng.normal(s) * 0.4)(D, 2 * Fh)), 'w_sp': _w(0.01 * (lambda *s: _rng.normal(s) * 0.4)(S, S)), 'b_sp': _w(1.0 + 0.01 * (lambda *s: _rng.normal(s) * 0.05)(S)), 'w_out': _w((lambda *s: _rng.normal(s) * 0.05)(Fh, D))}
    _B_in = _B_setup()
    return {'A_x': _A_in['x'], 'A_wqkv': _A_in['wqkv'], 'A_wo': _A_in['wo'], 'B_x': _B_in['x'], 'B_w_in': _B_in['w_in'], 'B_w_sp': _B_in['w_sp'], 'B_b_sp': _B_in['b_sp'], 'B_w_out': _B_in['w_out']}

def reference(A_x, A_wqkv, A_wo, B_x, B_w_in, B_w_sp, B_b_sp, B_w_out):

    def _A_ref(x, wqkv, wo):
        B, S, D = x.shape
        H = 32
        Dh = D // H
        qkv = (lambda x, *d: x.transpose(*d))((x @ wqkv).reshape(B, S, 3, H, Dh), 2, 0, 3, 1, 4)
        q, k, v = (qkv[0], qkv[1], qkv[2])
        phi = lambda t: jnp.where(t > 0, t + 1, jnp.exp(t)) + 1e-06
        pq, pk = (phi(q), phi(k))
        kv = jnp.einsum('bhsd,bhse->bhde', pk, v)
        z = jnp.einsum('bhsd->bhd', pk)
        num = jnp.einsum('bhqd,bhde->bhqe', pq, kv)
        den = jnp.einsum('bhqd,bhd->bhq', pq, z)[..., None] + 1e-06
        o = num / den
        return (lambda x, *d: x.transpose(*d))(o, 0, 2, 1, 3).reshape(B, S, D) @ wo

    def _B_ref(x, w_in, w_sp, b_sp, w_out):
        B, S, D = x.shape
        F = w_in.shape[-1]
        Fh = F // 2
        z = _gelu(jnp.einsum('bsd,df->bsf', x, w_in))
        z1 = z[..., :Fh].copy()
        z2 = _layernorm(z[..., Fh:], axis=-1)
        g = jnp.einsum('ts,bsf->btf', w_sp, z2) + b_sp[None, :, None]
        return jnp.einsum('bsf,fd->bsd', z1 * g, w_out)
    x = A_x
    h = x + _A_ref(_layernorm(x, axis=-1), A_wqkv, A_wo)
    h2 = h + _B_ref(_layernorm(h, axis=-1), B_w_in, B_w_sp, B_b_sp, B_w_out)
    return h2
```

```python
import functools
import jax
import jax.numpy as jnp
import jax.experimental.pallas as pl
import jax.experimental.pallas.tpu as pltpu

S, D, F = 2048, 512, 1792
FH = F // 2
DH = 16
BF = jnp.bfloat16
F32 = jnp.float32


def _ln(x, scale=None):
    m = jnp.mean(x, axis=-1, keepdims=True)
    xc = x - m
    v = jnp.mean(xc * xc, axis=-1, keepdims=True)
    r = jax.lax.rsqrt(v + 1e-5)
    if scale is not None:
        r = r * scale
    return xc * r


def _phi(t):
    return jnp.where(t > 0, t + 1.0, jnp.exp(t)) + 1e-6


def _gelu_half(y):
    c0 = 2.0 * 0.7978845608028654
    c1 = 8.0 * 0.7978845608028654 * 0.044715
    return y * jnp.tanh(y * (c0 + c1 * (y * y))) + y


def _recip(d):
    r = pl.reciprocal(d, approx=True)
    return r * (2.0 - d * r)


def _dot(a, b):
    return jnp.dot(a, b, preferred_element_type=F32)


def make_kernel(TM1, TM2, TM3, TO, unroll1, unroll2, unroll3, split2):
    n1, n2, n3 = S // TM1, S // TM2, S // TM3
    no = S // TO

    def kernel(x_hbm, wqkv_hbm, wo_hbm, win_hbm, wsp_hbm, bsp_hbm, wout_hbm, o_hbm,
               x_v, wqkv_v, wo_v, win_v, wsp_v, bsp_v, wout_v,
               xn_v, wkT_v, T_v, zacc_v, m_v, zb_v, h_v, hn_v, z1_v, z2_v, bcol_v, o_v, sx, sw, ssp, so):
        def rows(i, tm):
            if isinstance(i, int):
                return pl.ds(i * tm, tm)
            return pl.ds(pl.multiple_of(i * tm, tm), tm)

        def xc(i):
            return pltpu.make_async_copy(x_hbm.at[0, rows(i, TM1)], x_v.at[rows(i, TM1)], sx.at[i])

        def spc(i):
            return pltpu.make_async_copy(wsp_hbm.at[rows(i, TM3)], wsp_v.at[rows(i, TM3)], ssp.at[i])

        def oc(i):
            return pltpu.make_async_copy(o_v.at[rows(i, TO)], o_hbm.at[0, rows(i, TO)], so.at[i])

        wq_c = pltpu.make_async_copy(wqkv_hbm.at[:, pl.ds(0, D)], wqkv_v.at[0], sw.at[0])
        wk_c = pltpu.make_async_copy(wqkv_hbm.at[:, pl.ds(D, D)], wqkv_v.at[1], sw.at[1])
        wv_c = pltpu.make_async_copy(wqkv_hbm.at[:, pl.ds(2 * D, D)], wqkv_v.at[2], sw.at[2])
        wo_c = pltpu.make_async_copy(wo_hbm, wo_v, sw.at[3])
        win_c = pltpu.make_async_copy(win_hbm, win_v, sw.at[4])
        wout_c = pltpu.make_async_copy(wout_hbm, wout_v, sw.at[5])
        bsp_c = pltpu.make_async_copy(bsp_hbm, bsp_v, sw.at[6])

        xc(0).start()
        wk_c.start()
        if n1 > 1:
            xc(1).start()

        def ln1(i):
            r = rows(i, TM1)
            xn = _ln(x_v[r, :].astype(F32)).astype(BF)
            xn_v[r, :] = xn
            return xn

        def p1(xn):
            kT = jax.lax.dot_general(wkT_v[...], xn, (((1,), (1,)), ((), ())), preferred_element_type=F32)
            pk = _phi(kT)
            zs = pk[:, 0:128]
            for j in range(1, TM1 // 128):
                zs = zs + pk[:, j * 128:(j + 1) * 128]
            zacc_v[...] += zs
            T_v[...] += _dot(pk.astype(BF), xn)

        xc(0).wait()
        xn0 = ln1(0)
        T_v[...] = jnp.zeros((D, D), F32)
        zacc_v[...] = jnp.zeros((D, 128), F32)
        wk_c.wait()
        for i in range(2, n1):
            xc(i).start()
        wv_c.start()
        wo_c.start()
        wq_c.start()
        win_c.start()
        wkT_v[...] = wqkv_v[1].T

        def body1(i, xn):
            xc(i + 1).wait()
            xn_next = ln1(i + 1)
            p1(xn)
            return xn_next

        xn_last = jax.lax.fori_loop(0, n1 - 1, body1, xn0, unroll=unroll1)
        bsp_c.start()
        wout_c.start()
        for i in range(n3):
            spc(i).start()
        wv_c.wait()
        wo_c.wait()
        wq_c.wait()
        win_c.wait()
        p1(xn_last)

        def qproj(i):
            return _phi(_dot(xn_v[rows(i, TM2), :], wqkv_v[0]))

        def scale_q(pq):
            parts = []
            dens = [_dot(pq[:, g * 128:(g + 1) * 128].astype(BF), zb_v[g]) + 1e-6 for g in range(4)]
            for g in range(4):
                parts.append((pq[:, g * 128:(g + 1) * 128] * _recip(dens[g])).astype(BF))
            return jnp.concatenate(parts, axis=1)

        def attn_out(i, a):
            r = rows(i, TM2)
            h = x_v[r, :].astype(F32) + _dot(a, m_v[...])
            h_v[r, :] = h
            return _ln(h, 0.5).astype(BF)

        z = jnp.sum(zacc_v[...], axis=1, keepdims=True)
        ri = jax.lax.broadcasted_iota(jnp.int32, (128, 128), 0) // DH
        ci = jax.lax.broadcasted_iota(jnp.int32, (128, 128), 1) // DH
        mask = ri == ci
        for g in range(4):
            gs = slice(g * 128, (g + 1) * 128)
            zb_v[g] = jnp.where(mask, z[gs, :], 0.0).astype(BF)
        pq0 = qproj(0)
        kvs = []
        for g in range(4):
            gs = slice(g * 128, (g + 1) * 128)
            kv = _dot(T_v[gs, :].astype(BF), wqkv_v[2, :, gs])
            kvs.append(jnp.where(mask, kv, 0.0).astype(BF))
        a0 = scale_q(pq0)
        for g in range(4):
            gs = slice(g * 128, (g + 1) * 128)
            m_v[gs, :] = _dot(kvs[g], wo_v[gs, :]).astype(BF)
        hn0 = attn_out(0, a0)

        c1 = FH + 128 * split2

        def finish_z2(i, z2a, z2b):
            z2_v[rows(i, TM2), :] = _ln(_gelu_half(jnp.concatenate([z2a, z2b], axis=1))).astype(BF)

        def body2(i, hn):
            pq = qproj(i + 1)
            z2a = _dot(hn, win_v[:, FH:c1])
            a = scale_q(pq)
            z2b = _dot(hn, win_v[:, c1:])
            hn_next = attn_out(i + 1, a)
            finish_z2(i, z2a, z2b)
            z1_v[rows(i, TM2), :] = _gelu_half(_dot(hn, win_v[:, :FH])).astype(BF)
            return hn_next

        hn_last = jax.lax.fori_loop(0, n2 - 1, body2, hn0, unroll=unroll2)

        bsp_c.wait()
        for j in range(S // 128):
            brow = bsp_v[pl.ds(j * 128, 128)].astype(F32).reshape(1, 128)
            bcol_v[pl.ds(j * 128, 128), :] = jnp.broadcast_to(brow, (128, 128)).T
        z2_v[rows(n2 - 1, TM2), :] = _ln(_gelu_half(_dot(hn_last, win_v[:, FH:]))).astype(BF)
        z1_v[rows(n2 - 1, TM2), :] = _gelu_half(_dot(hn_last, win_v[:, :FH])).astype(BF)

        wout_c.wait()

        def stage_c(i):
            r = rows(i, TM3)
            spc(i).wait()
            g = _dot(wsp_v[r, :], z2_v[...])
            bcol = bcol_v[r, :]
            gb = g + jnp.concatenate([bcol] * 7, axis=1)
            u = (z1_v[r, :].astype(F32) * gb).astype(BF)
            o_v[r, :] = (h_v[r, :] + _dot(u, wout_v[...])).astype(BF)
            for k in range(TM3 // TO):
                oc(i * (TM3 // TO) + k).start()

        def body3(i, c):
            stage_c(i)
            return c

        jax.lax.fori_loop(0, n3, body3, 0, unroll=unroll3)
        for i in range(no):
            oc(i).wait()

    return kernel, n1, n3, no


def build(TM1=512, TM2=256, TM3=512, TO=None, unroll1=False, unroll2=False, unroll3=False, split2=3, **kw):
    TO = TO or TM3
    kernel, n1, n3, no = make_kernel(TM1, TM2, TM3, TO, unroll1, unroll2, unroll3, split2)

    @jax.jit
    def fn(A_x, A_wqkv, A_wo, B_x, B_w_in, B_w_sp, B_b_sp, B_w_out):
        any_spec = pl.BlockSpec(memory_space=pl.ANY)
        return pl.pallas_call(
            kernel,
            out_shape=jax.ShapeDtypeStruct((1, S, D), BF),
            in_specs=[any_spec] * 7,
            out_specs=any_spec,
            scratch_shapes=[
                pltpu.VMEM((S, D), BF),
                pltpu.VMEM((3, D, D), BF),
                pltpu.VMEM((D, D), BF),
                pltpu.VMEM((D, F), BF),
                pltpu.VMEM((S, S), BF),
                pltpu.VMEM((S,), BF),
                pltpu.VMEM((FH, D), BF),
                pltpu.VMEM((S, D), BF),
                pltpu.VMEM((D, D), BF),
                pltpu.VMEM((D, D), F32),
                pltpu.VMEM((D, 128), F32),
                pltpu.VMEM((D, D), BF),
                pltpu.VMEM((4, 128, 128), BF),
                pltpu.VMEM((S, D), F32),
                pltpu.VMEM((S, D), BF),
                pltpu.VMEM((S, FH), BF),
                pltpu.VMEM((S, FH), BF),
                pltpu.VMEM((S, 128), F32),
                pltpu.VMEM((S, D), BF),
                pltpu.SemaphoreType.DMA((n1,)),
                pltpu.SemaphoreType.DMA((7,)),
                pltpu.SemaphoreType.DMA((n3,)),
                pltpu.SemaphoreType.DMA((no,)),
            ],
            compiler_params=pltpu.CompilerParams(vmem_limit_bytes=100 * 2**20, **({"flags": kw["flags"]} if "flags" in kw else {})),
        )(A_x, A_wqkv, A_wo, B_w_in, B_w_sp, B_b_sp, B_w_out)

    return fn


_impl = build(**dict())


def pallas_sequential_preLN__linear_attn_block__mixer_gmlp__prompt_kernel(
    A_x, A_wqkv, A_wo, B_x, B_w_in, B_w_sp, B_b_sp, B_w_out
):
    return _impl(A_x, A_wqkv, A_wo, B_x, B_w_in, B_w_sp, B_b_sp, B_w_out)
```

```python
import jax
import jax.numpy as jnp
import jax.experimental.pallas as pl
import jax.experimental.pallas.tpu as pltpu

S, D, F = 2048, 512, 1792
FH = F // 2
DH = 16
H2 = S // 2
NH = 384
C0 = 2 * NH
DH2 = D // 2
BF = jnp.bfloat16
F32 = jnp.float32


def _ln(x, scale=None):
    m = jnp.mean(x, axis=-1, keepdims=True)
    xc = x - m
    v = jnp.mean(xc * xc, axis=-1, keepdims=True)
    r = jax.lax.rsqrt(v + 1e-5)
    if scale is not None:
        r = r * scale
    return xc * r


def _phi(t):
    return jnp.where(t > 0, t + 1.0, jnp.exp(t)) + 1e-6


def _gelu_of_double(y):
    c0 = 2.0 * 0.7978845608028654
    c1 = 8.0 * 0.7978845608028654 * 0.044715
    return y * jnp.tanh(y * (c0 + c1 * (y * y))) + y


def _recip(d):
    r = pl.reciprocal(d, approx=True)
    return r * (2.0 - d * r)


def _dot(a, b):
    return jnp.dot(a, b, preferred_element_type=F32)


def _dot_nt(a, b):
    return jax.lax.dot_general(a, b, (((1,), (1,)), ((), ())), preferred_element_type=F32)


def _add_bf(x, y):
    return (x.astype(F32) + y.astype(F32)).astype(BF)


def _sub_bf(x, y):
    return (x.astype(F32) - y.astype(F32)).astype(BF)


def make_kernel(TM1, X0, TM2, SEG, TR, TO, WC, OPT):
    n1, n2, n3 = S // TM1, S // TM2, H2 // TR
    nx0 = TM1 // X0
    npair = TM2 // (2 * SEG)

    def kernel(x_hbm, wqkv_hbm, wo_hbm, win_hbm, wsp_hbm, bsp_hbm, wout_hbm, o_hbm,
               x_v, wqkv_v, wo_v, win_v, wsp_v, bsp_v, wout_v,
               xn_v, wkT_v, wqT_v, pk_v, T_v, zacc_v, zcol_v, m_v, h_v, hn_v,
               z1_v, b_v, wb_v, zr_v, bcol_v, o_v,
               sx0, sx, sw, ssp, so):
        def rows(i, tm):
            if isinstance(i, int):
                return pl.ds(i * tm, tm)
            return pl.ds(pl.multiple_of(i * tm, tm), tm)

        def top(i, k):
            return rows(i * npair + k, SEG)

        def bot(i, k):
            return rows(H2 // SEG + i * npair + k, SEG)

        def segs(i):
            return [f(i, k) for k in range(npair) for f in (top, bot)]

        def x0c(c):
            return pltpu.make_async_copy(x_hbm.at[0, rows(c, X0)], x_v.at[rows(c, X0)], sx0.at[c])

        def xc(i):
            return pltpu.make_async_copy(x_hbm.at[0, rows(i, TM1)], x_v.at[rows(i, TM1)], sx.at[i])

        def spc(i):
            return pltpu.make_async_copy(wsp_hbm.at[rows(i, TR)], wsp_v.at[rows(i, TR)], ssp.at[i])

        def oc(i):
            return pltpu.make_async_copy(o_v.at[rows(i, TO)], o_hbm.at[0, rows(i, TO)], so.at[0])

        wk_c = pltpu.make_async_copy(wqkv_hbm.at[:, pl.ds(D, D)], wqkv_v.at[1], sw.at[0])
        bsp_c = pltpu.make_async_copy(bsp_hbm, bsp_v, sw.at[1])
        wq_c = pltpu.make_async_copy(wqkv_hbm.at[:, pl.ds(0, D)], wqkv_v.at[0], sw.at[2])
        wv_c = pltpu.make_async_copy(wqkv_hbm.at[:, pl.ds(2 * D, D)], wqkv_v.at[2], sw.at[3])
        wo_c = pltpu.make_async_copy(wo_hbm, wo_v, sw.at[4])
        win_c = pltpu.make_async_copy(win_hbm, win_v, sw.at[5])
        wout_c = pltpu.make_async_copy(wout_hbm, wout_v, sw.at[6])

        bsp_c.start()
        x0c(0).start()
        wk_c.start()
        for c in range(1, nx0):
            x0c(c).start()
        T_v[...] = jnp.zeros((D, D), F32)
        bsp_c.wait()
        for j in range(S // 128):
            brow = bsp_v[pl.ds(j * 128, 128)].astype(F32).reshape(1, 128)
            bcol_v[pl.ds(j * 128, 128), :] = jnp.broadcast_to(brow, (128, 128)).T

        def ln_x(r):
            xn = _ln(x_v[r, :].astype(F32)).astype(BF)
            xn_v[r, :] = xn
            return xn

        def lane_sum(pk):
            zs = pk[:, 0:128]
            for j in range(1, pk.shape[1] // 128):
                zs = zs + pk[:, j * 128:(j + 1) * 128]
            return zs

        def t_acc(i):
            T_v[...] += _dot(pk_v[...], xn_v[rows(i, TM1), :])

        x0c(0).wait()
        xc(1).start()
        xn = ln_x(rows(0, X0))
        wk_c.wait()
        wkT = wqkv_v[1].T
        wkT_v[...] = wkT
        zs = None
        for c in range(nx0):
            if c + 1 < nx0:
                x0c(c + 1).wait()
                xn_next = ln_x(rows(c + 1, X0))
            pk = _phi(_dot_nt(wkT, xn))
            pk_v[:, c * X0:(c + 1) * X0] = pk.astype(BF)
            zs = lane_sum(pk) if zs is None else zs + lane_sum(pk)
            if c + 1 < nx0:
                xn = xn_next
        zacc_v[...] = zs

        def body1(i, carry):
            xc(i + 1).wait()

            @pl.when(i + 2 < n1)
            def _():
                xc(i + 2).start()

            @pl.when(i == 0)
            def _():
                wq_c.start()

            @pl.when(i == 1)
            def _():
                wv_c.start()
                wo_c.start()
                win_c.start()

            t_acc(i)
            pk = _phi(_dot_nt(wkT_v[...], ln_x(rows(i + 1, TM1))))
            zacc_v[...] += lane_sum(pk)
            pk_v[...] = pk.astype(BF)
            return carry

        jax.lax.fori_loop(0, n1 - 1, body1, 0)
        wout_c.start()
        for i in range(2 * n3):
            spc(i).start()
        wv_c.wait()
        wo_c.wait()
        wq_c.wait()
        wqT_v[...] = wqkv_v[0].T
        t_acc(n1 - 1)

        def q_proj(i):
            xn = jnp.concatenate([xn_v[r, :] for r in segs(i)], axis=0)
            return _phi(_dot_nt(wqT_v[...], xn))

        def scale_q(pqT):
            zcol = zcol_v[...].reshape(D // DH, DH, 128)
            outs = []
            for j in range(TM2 // 128):
                p = pqT[:, j * 128:(j + 1) * 128].reshape(D // DH, DH, 128)
                den = jnp.sum(p * zcol, axis=1, keepdims=True) + 1e-6
                outs.append((p * _recip(den)).reshape(D, 128))
            return jnp.concatenate(outs, axis=1).astype(BF).T

        def attn_out(i, a):
            x = jnp.concatenate([x_v[r, :] for r in segs(i)], axis=0)
            h = x.astype(F32) + _dot(a, m_v[...])
            for c in range(0, D, 128):
                for s, r in enumerate(segs(i)):
                    h_v[r, c:c + 128] = h[s * SEG:(s + 1) * SEG, c:c + 128]
            hn_v[...] = _ln(h, 0.5).astype(BF)

        z = jnp.sum(zacc_v[...], axis=1, keepdims=True)
        zcol_v[...] = jnp.broadcast_to(z, (D, 128))
        same_head = (jax.lax.broadcasted_iota(jnp.int32, (128, 128), 0) // DH
                     == jax.lax.broadcasted_iota(jnp.int32, (128, 128), 1) // DH)
        pq0 = q_proj(0)
        kvs = []
        for g in range(0, D, 128):
            kv = _dot(T_v[g:g + 128, :].astype(BF), wqkv_v[2, :, g:g + 128])
            kvs.append(jnp.where(same_head, kv, 0.0).astype(BF))
        a0 = scale_q(pq0)
        for j, g in enumerate(range(0, D, 128)):
            m_v[g:g + 128, :] = _dot(kvs[j], wo_v[g:g + 128, :]).astype(BF)
        attn_out(0, a0)

        def z_act(hn, lo, hi):
            return _gelu_of_double(_dot(hn, win_v[:, lo:hi]))

        def z2_pair(i, hn, k):
            zz = _ln(z_act(hn[2 * k * SEG:(2 * k + 2) * SEG, :], FH, F))
            b11, b12, b21, b22 = zz[:SEG, :NH], zz[:SEG, NH:C0], zz[SEG:, :NH], zz[SEG:, NH:C0]
            t = top(i, k)
            b_v[0, t, :] = (b11 + b22).astype(BF)
            b_v[1, t, :] = b11.astype(BF)
            b_v[2, t, :] = (b12 - b22).astype(BF)
            b_v[3, t, :] = (b21 - b11).astype(BF)
            b_v[4, t, :] = b22.astype(BF)
            b_v[5, t, :] = (b11 + b12).astype(BF)
            b_v[6, t, :] = (b21 + b22).astype(BF)
            zr_v[t, :] = zz[:SEG, C0:].astype(BF)
            zr_v[bot(i, k), :] = zz[SEG:, C0:].astype(BF)

        def z1_tile(i, hn):
            for c in range(0, FH, 128):
                z1 = z_act(hn, c, c + 128).astype(BF)
                for s, r in enumerate(segs(i)):
                    z1_v[r, c:c + 128] = z1[s * SEG:(s + 1) * SEG, :]

        def body2(i, carry):
            hn = hn_v[...]
            pq = q_proj(i + 1)
            z2_pair(i, hn, 0)
            a = scale_q(pq)
            for k in range(1, npair):
                z2_pair(i, hn, k)
            attn_out(i + 1, a)
            z1_tile(i, hn)
            return carry

        win_c.wait()
        jax.lax.fori_loop(0, n2 - 1, body2, 0)

        wout_c.wait()
        for r in range(0, NH, WC):
            lo, hi = pl.ds(r, WC), pl.ds(NH + r, WC)
            w11, w12 = wout_v[lo, 0:DH2], wout_v[lo, DH2:D]
            w21, w22 = wout_v[hi, 0:DH2], wout_v[hi, DH2:D]
            wb_v[0, lo, :] = _add_bf(w11, w22)
            wb_v[1, lo, :] = _sub_bf(w12, w22)
            wb_v[2, lo, :] = _sub_bf(w21, w11)
            wb_v[3, lo, :] = _add_bf(w11, w12)
            wb_v[4, lo, :] = _add_bf(w21, w22)
        hn_last = hn_v[...]
        for k in range(npair):
            z2_pair(n2 - 1, hn_last, k)
        z1_tile(n2 - 1, hn_last)

        for i in range(2 * n3):
            spc(i).wait()

        def body3(i, carry):
            t = rows(i, TR)
            u = rows(i + n3, TR)
            a11, a12 = wsp_v[t, 0:H2], wsp_v[t, H2:S]
            a21, a22 = wsp_v[u, 0:H2], wsp_v[u, H2:S]
            bt, bu = bcol_v[t, :], bcol_v[u, :]

            m3 = _dot(a11, b_v[2])
            m1 = _dot(_add_bf(a11, a22), b_v[0])
            m2 = _dot(_add_bf(a21, a22), b_v[1])
            m4 = _dot(a22, b_v[3])
            c21 = m2 + m4
            m6 = _dot(_sub_bf(a21, a11), b_v[5])
            c22 = (m1 - m2) + (m3 + m6)
            ru = _dot(jnp.concatenate([a21, a22], axis=1), zr_v[...]) + bu
            m5 = _dot(_add_bf(a11, a12), b_v[4])
            c12 = m3 + m5
            m7 = _dot(_sub_bf(a12, a22), b_v[6])
            c11 = (m1 + m4) + (m7 - m5)
            rt = _dot(jnp.concatenate([a11, a12], axis=1), zr_v[...]) + bt

            def gate(r, c1, c2, cr, b):
                b3 = jnp.concatenate([b] * (NH // 128), axis=1)
                g = jnp.concatenate([c1 + b3, c2 + b3, cr], axis=1)
                return z1_v[r, :].astype(F32) * g

            ub = gate(u, c21, c22, ru, bu)
            ut = gate(t, c11, c12, rt, bt)
            nc = TR // TO
            for k in range(nc):
                p = ut[k * TO:(k + 1) * TO, :]
                q = ub[k * TO:(k + 1) * TO, :]
                u11, u12, u21, u22 = p[:, 0:NH], p[:, NH:C0], q[:, 0:NH], q[:, NH:C0]
                it, ib = i * nc + k, (i + n3) * nc + k
                ot, ob = rows(it, TO), rows(ib, TO)
                wr = wout_v[C0:FH, :]
                et = h_v[ot, :] + _dot(p[:, C0:FH].astype(BF), wr)
                eb = h_v[ob, :] + _dot(q[:, C0:FH].astype(BF), wr)
                s3 = _dot(u11.astype(BF), wb_v[1])
                s5 = _dot((u11 + u12).astype(BF), wout_v[NH:C0, DH2:D])
                o_v[ot, DH2:D] = (et[:, DH2:D] + (s3 + s5)).astype(BF)
                s2 = _dot((u21 + u22).astype(BF), wout_v[0:NH, 0:DH2])
                s1 = _dot((u11 + u22).astype(BF), wb_v[0])
                s6 = _dot((u21 - u11).astype(BF), wb_v[3])
                o_v[ob, DH2:D] = (eb[:, DH2:D] + ((s1 - s2) + (s3 + s6))).astype(BF)
                s4 = _dot(u22.astype(BF), wb_v[2])
                o_v[ob, 0:DH2] = (eb[:, 0:DH2] + (s2 + s4)).astype(BF)
                oc(ib).start()
                s7 = _dot((u12 - u22).astype(BF), wb_v[4])
                o_v[ot, 0:DH2] = (et[:, 0:DH2] + ((s1 + s4) + (s7 - s5))).astype(BF)
                oc(it).start()
            return carry

        jax.lax.fori_loop(0, n3, body3, 0)
        for i in range(S // TO):
            oc(i).wait()

    return kernel, n1, n3, nx0


def build(TM1=512, X0=256, TM2=512, SEG=64, TR=512, TO=128, WC=32, OPT=0):
    kernel, n1, n3, nx0 = make_kernel(TM1, X0, TM2, SEG, TR, TO, WC, OPT)

    @jax.jit
    def pallas_sequential_preLN__linear_attn_block__mixer_gmlp__prompt_kernel(
            A_x, A_wqkv, A_wo, B_x, B_w_in, B_w_sp, B_b_sp, B_w_out):
        del B_x
        any_spec = pl.BlockSpec(memory_space=pl.ANY)
        return pl.pallas_call(
            kernel,
            out_shape=jax.ShapeDtypeStruct((1, S, D), BF),
            in_specs=[any_spec] * 7,
            out_specs=any_spec,
            scratch_shapes=[
                pltpu.VMEM((S, D), BF),
                pltpu.VMEM((3, D, D), BF),
                pltpu.VMEM((D, D), BF),
                pltpu.VMEM((D, F), BF),
                pltpu.VMEM((S, S), BF),
                pltpu.VMEM((S,), BF),
                pltpu.VMEM((FH, D), BF),
                pltpu.VMEM((S, D), BF),
                pltpu.VMEM((D, D), BF),
                pltpu.VMEM((D, D), BF),
                pltpu.VMEM((D, TM1), BF),
                pltpu.VMEM((D, D), F32),
                pltpu.VMEM((D, 128), F32),
                pltpu.VMEM((D, 128), F32),
                pltpu.VMEM((D, D), BF),
                pltpu.VMEM((S, D), F32),
                pltpu.VMEM((TM2, D), BF),
                pltpu.VMEM((S, FH), BF),
                pltpu.VMEM((7, H2, NH), BF),
                pltpu.VMEM((5, NH, DH2), BF),
                pltpu.VMEM((S, 128), BF),
                pltpu.VMEM((S, 128), F32),
                pltpu.VMEM((S, D), BF),
                pltpu.SemaphoreType.DMA((nx0,)),
                pltpu.SemaphoreType.DMA((n1,)),
                pltpu.SemaphoreType.DMA((7,)),
                pltpu.SemaphoreType.DMA((2 * n3,)),
                pltpu.SemaphoreType.DMA((1,)),
            ],
            compiler_params=pltpu.CompilerParams(vmem_limit_bytes=100 * 2**20),
        )(A_x, A_wqkv, A_wo, B_w_in, B_w_sp, B_b_sp, B_w_out)

    return pallas_sequential_preLN__linear_attn_block__mixer_gmlp__prompt_kernel


pallas_sequential_preLN__linear_attn_block__mixer_gmlp__prompt_kernel = build(**dict())
```

```python
import jax
import jax.numpy as jnp
import jax.experimental.pallas as pl
import jax.experimental.pallas.tpu as pltpu

S, D, F = 2048, 512, 1792
FH = F // 2
DH = 16
H2 = S // 2
NH = 384
C0 = 2 * NH
DH2 = D // 2
BF = jnp.bfloat16
F32 = jnp.float32


def _ln(x, scale=None):
    m = jnp.mean(x, axis=-1, keepdims=True)
    xc = x - m
    v = jnp.mean(xc * xc, axis=-1, keepdims=True)
    r = jax.lax.rsqrt(v + 1e-5)
    if scale is not None:
        r = r * scale
    return xc * r


def _phi(t):
    return jnp.where(t > 0, t + 1.0, jnp.exp(t)) + 1e-6


def _gelu_of_double(y):
    c0 = 2.0 * 0.7978845608028654
    c1 = 8.0 * 0.7978845608028654 * 0.044715
    return y * jnp.tanh(y * (c0 + c1 * (y * y))) + y


def _recip(d):
    r = pl.reciprocal(d, approx=True)
    return r * (2.0 - d * r)


def _dot(a, b):
    return jnp.dot(a, b, preferred_element_type=F32)


def _dot_nt(a, b):
    return jax.lax.dot_general(a, b, (((1,), (1,)), ((), ())), preferred_element_type=F32)


def _add_bf(x, y):
    return (x.astype(F32) + y.astype(F32)).astype(BF)


def _sub_bf(x, y):
    return (x.astype(F32) - y.astype(F32)).astype(BF)


def make_kernel(TM1, X0, TM2, SEG, TR, TO, WC):
    n1, n2, n3 = S // TM1, S // TM2, H2 // TR
    nx0 = TM1 // X0
    npair = TM2 // (2 * SEG)

    def kernel(x_hbm, wqkv_hbm, wo_hbm, win_hbm, wsp_hbm, bsp_hbm, wout_hbm, o_hbm,
               x_v, wqkv_v, wo_v, win_v, wsp_v, bsp_v, wout_v,
               xn_v, wkT_v, wqT_v, pk_v, T_v, zacc_v, zcol_v, m_v, h_v, hn_v,
               z1_v, b_v, wb_v, zr_v, bcol_v, o_v,
               sx0, sx, sw, ssp, so):
        def rows(i, tm):
            if isinstance(i, int):
                return pl.ds(i * tm, tm)
            return pl.ds(pl.multiple_of(i * tm, tm), tm)

        def top(i, k):
            return rows(i * npair + k, SEG)

        def bot(i, k):
            return rows(H2 // SEG + i * npair + k, SEG)

        def segs(i):
            return [f(i, k) for k in range(npair) for f in (top, bot)]

        def x0c(c):
            return pltpu.make_async_copy(x_hbm.at[0, rows(c, X0)], x_v.at[rows(c, X0)], sx0.at[c])

        def xc(i):
            return pltpu.make_async_copy(x_hbm.at[0, rows(i, TM1)], x_v.at[rows(i, TM1)], sx.at[i])

        def spc(i):
            return pltpu.make_async_copy(wsp_hbm.at[rows(i, TR)], wsp_v.at[rows(i, TR)], ssp.at[i])

        def oc(i):
            return pltpu.make_async_copy(o_v.at[rows(i, TO)], o_hbm.at[0, rows(i, TO)], so.at[0])

        wk_c = pltpu.make_async_copy(wqkv_hbm.at[:, pl.ds(D, D)], wqkv_v.at[1], sw.at[0])
        bsp_c = pltpu.make_async_copy(bsp_hbm, bsp_v, sw.at[1])
        wq_c = pltpu.make_async_copy(wqkv_hbm.at[:, pl.ds(0, D)], wqkv_v.at[0], sw.at[2])
        wv_c = pltpu.make_async_copy(wqkv_hbm.at[:, pl.ds(2 * D, D)], wqkv_v.at[2], sw.at[3])
        wo_c = pltpu.make_async_copy(wo_hbm, wo_v, sw.at[4])
        win_c = pltpu.make_async_copy(win_hbm, win_v, sw.at[5])
        wout_c = pltpu.make_async_copy(wout_hbm, wout_v, sw.at[6])

        bsp_c.start()
        x0c(0).start()
        wk_c.start()
        for c in range(1, nx0):
            x0c(c).start()
        T_v[...] = jnp.zeros((D, D), F32)
        bsp_c.wait()
        for j in range(S // 128):
            brow = bsp_v[pl.ds(j * 128, 128)].astype(F32).reshape(1, 128)
            bcol_v[pl.ds(j * 128, 128), :] = jnp.broadcast_to(brow, (128, 128)).T

        def ln_x(r):
            xn = _ln(x_v[r, :].astype(F32)).astype(BF)
            xn_v[r, :] = xn
            return xn

        def lane_sum(pk):
            zs = pk[:, 0:128]
            for j in range(1, pk.shape[1] // 128):
                zs = zs + pk[:, j * 128:(j + 1) * 128]
            return zs

        def t_acc(i):
            T_v[...] += _dot(pk_v[...], xn_v[rows(i, TM1), :])

        x0c(0).wait()
        xc(1).start()
        xn = ln_x(rows(0, X0))
        wk_c.wait()
        wkT = wqkv_v[1].T
        wkT_v[...] = wkT
        zs = None
        for c in range(nx0):
            if c + 1 < nx0:
                x0c(c + 1).wait()
                xn_next = ln_x(rows(c + 1, X0))
            pk = _phi(_dot_nt(wkT, xn))
            pk_v[:, c * X0:(c + 1) * X0] = pk.astype(BF)
            zs = lane_sum(pk) if zs is None else zs + lane_sum(pk)
            if c + 1 < nx0:
                xn = xn_next
        zacc_v[...] = zs

        def body1(i, carry):
            xc(i + 1).wait()

            @pl.when(i + 2 < n1)
            def _():
                xc(i + 2).start()

            @pl.when(i == 0)
            def _():
                wq_c.start()

            @pl.when(i == 1)
            def _():
                wv_c.start()
                wo_c.start()
                win_c.start()

            t_acc(i)
            pk = _phi(_dot_nt(wkT_v[...], ln_x(rows(i + 1, TM1))))
            zacc_v[...] += lane_sum(pk)
            pk_v[...] = pk.astype(BF)
            return carry

        jax.lax.fori_loop(0, n1 - 1, body1, 0)
        wout_c.start()
        for i in range(2 * n3):
            spc(i).start()
        wv_c.wait()
        wo_c.wait()
        wq_c.wait()
        wqT_v[...] = wqkv_v[0].T
        t_acc(n1 - 1)

        def q_proj(i):
            xn = jnp.concatenate([xn_v[r, :] for r in segs(i)], axis=0)
            return _phi(_dot_nt(wqT_v[...], xn))

        def scale_q(pqT):
            zcol = zcol_v[...].reshape(D // DH, DH, 128)
            outs = []
            for j in range(TM2 // 128):
                p = pqT[:, j * 128:(j + 1) * 128].reshape(D // DH, DH, 128)
                den = jnp.sum(p * zcol, axis=1, keepdims=True) + 1e-6
                outs.append((p * _recip(den)).reshape(D, 128))
            return jnp.concatenate(outs, axis=1).astype(BF).T

        def attn_out(i, a):
            x = jnp.concatenate([x_v[r, :] for r in segs(i)], axis=0)
            h = x.astype(F32) + _dot(a, m_v[...])
            for c in range(0, D, 128):
                for s, r in enumerate(segs(i)):
                    h_v[r, c:c + 128] = h[s * SEG:(s + 1) * SEG, c:c + 128]
            hn_v[...] = _ln(h, 0.5).astype(BF)

        z = jnp.sum(zacc_v[...], axis=1, keepdims=True)
        zcol_v[...] = jnp.broadcast_to(z, (D, 128))
        same_head = (jax.lax.broadcasted_iota(jnp.int32, (128, 128), 0) // DH
                     == jax.lax.broadcasted_iota(jnp.int32, (128, 128), 1) // DH)
        pq0 = q_proj(0)
        kvs = []
        for g in range(0, D, 128):
            kv = _dot(T_v[g:g + 128, :].astype(BF), wqkv_v[2, :, g:g + 128])
            kvs.append(jnp.where(same_head, kv, 0.0).astype(BF))
        a0 = scale_q(pq0)
        for j, g in enumerate(range(0, D, 128)):
            m_v[g:g + 128, :] = _dot(kvs[j], wo_v[g:g + 128, :]).astype(BF)
        attn_out(0, a0)

        def z_act(hn, lo, hi):
            return _gelu_of_double(_dot(hn, win_v[:, lo:hi]))

        def z2_pair(i, hn, k):
            zz = _ln(z_act(hn[2 * k * SEG:(2 * k + 2) * SEG, :], FH, F))
            b11, b12, b21, b22 = zz[:SEG, :NH], zz[:SEG, NH:C0], zz[SEG:, :NH], zz[SEG:, NH:C0]
            t = top(i, k)
            b_v[0, t, :] = (b11 + b22).astype(BF)
            b_v[1, t, :] = b11.astype(BF)
            b_v[2, t, :] = (b12 - b22).astype(BF)
            b_v[3, t, :] = (b21 - b11).astype(BF)
            b_v[4, t, :] = b22.astype(BF)
            b_v[5, t, :] = (b11 + b12).astype(BF)
            b_v[6, t, :] = (b21 + b22).astype(BF)
            zr_v[t, :] = zz[:SEG, C0:].astype(BF)
            zr_v[bot(i, k), :] = zz[SEG:, C0:].astype(BF)

        def z1_tile(i, hn):
            for c in range(0, FH, 128):
                z1 = z_act(hn, c, c + 128).astype(BF)
                for s, r in enumerate(segs(i)):
                    z1_v[r, c:c + 128] = z1[s * SEG:(s + 1) * SEG, :]

        def body2(i, carry):
            hn = hn_v[...]
            pq = q_proj(i + 1)
            z2_pair(i, hn, 0)
            a = scale_q(pq)
            for k in range(1, npair):
                z2_pair(i, hn, k)
            attn_out(i + 1, a)
            z1_tile(i, hn)
            return carry

        win_c.wait()
        jax.lax.fori_loop(0, n2 - 1, body2, 0)

        wout_c.wait()
        for r in range(0, NH, WC):
            lo, hi = pl.ds(r, WC), pl.ds(NH + r, WC)
            w11, w12 = wout_v[lo, 0:DH2], wout_v[lo, DH2:D]
            w21, w22 = wout_v[hi, 0:DH2], wout_v[hi, DH2:D]
            wb_v[0, lo, :] = _add_bf(w11, w22)
            wb_v[1, lo, :] = _sub_bf(w12, w22)
            wb_v[2, lo, :] = _sub_bf(w21, w11)
            wb_v[3, lo, :] = _add_bf(w11, w12)
            wb_v[4, lo, :] = _add_bf(w21, w22)
        hn_last = hn_v[...]
        for k in range(npair):
            z2_pair(n2 - 1, hn_last, k)
        z1_tile(n2 - 1, hn_last)

        for i in range(2 * n3):
            spc(i).wait()

        def body3(i, carry):
            t = rows(i, TR)
            u = rows(i + n3, TR)
            a11, a12 = wsp_v[t, 0:H2], wsp_v[t, H2:S]
            a21, a22 = wsp_v[u, 0:H2], wsp_v[u, H2:S]
            bt, bu = bcol_v[t, :], bcol_v[u, :]

            m3 = _dot(a11, b_v[2])
            m1 = _dot(_add_bf(a11, a22), b_v[0])
            m2 = _dot(_add_bf(a21, a22), b_v[1])
            m4 = _dot(a22, b_v[3])
            c21 = m2 + m4
            m6 = _dot(_sub_bf(a21, a11), b_v[5])
            c22 = (m1 - m2) + (m3 + m6)
            ru = _dot(jnp.concatenate([a21, a22], axis=1), zr_v[...]) + bu
            m5 = _dot(_add_bf(a11, a12), b_v[4])
            c12 = m3 + m5
            m7 = _dot(_sub_bf(a12, a22), b_v[6])
            c11 = (m1 + m4) + (m7 - m5)
            rt = _dot(jnp.concatenate([a11, a12], axis=1), zr_v[...]) + bt

            def gate(r, c1, c2, cr, b):
                b3 = jnp.concatenate([b] * (NH // 128), axis=1)
                g = jnp.concatenate([c1 + b3, c2 + b3, cr], axis=1)
                return z1_v[r, :].astype(F32) * g

            ub = gate(u, c21, c22, ru, bu)
            ut = gate(t, c11, c12, rt, bt)
            nc = TR // TO
            for k in range(nc):
                p = ut[k * TO:(k + 1) * TO, :]
                q = ub[k * TO:(k + 1) * TO, :]
                u11, u12, u21, u22 = p[:, 0:NH], p[:, NH:C0], q[:, 0:NH], q[:, NH:C0]
                it, ib = i * nc + k, (i + n3) * nc + k
                ot, ob = rows(it, TO), rows(ib, TO)
                wr = wout_v[C0:FH, :]
                et = h_v[ot, :] + _dot(p[:, C0:FH].astype(BF), wr)
                eb = h_v[ob, :] + _dot(q[:, C0:FH].astype(BF), wr)
                s3 = _dot(u11.astype(BF), wb_v[1])
                s5 = _dot((u11 + u12).astype(BF), wout_v[NH:C0, DH2:D])
                o_v[ot, DH2:D] = (et[:, DH2:D] + (s3 + s5)).astype(BF)
                s2 = _dot((u21 + u22).astype(BF), wout_v[0:NH, 0:DH2])
                s1 = _dot((u11 + u22).astype(BF), wb_v[0])
                s6 = _dot((u21 - u11).astype(BF), wb_v[3])
                o_v[ob, DH2:D] = (eb[:, DH2:D] + ((s1 - s2) + (s3 + s6))).astype(BF)
                s4 = _dot(u22.astype(BF), wb_v[2])
                o_v[ob, 0:DH2] = (eb[:, 0:DH2] + (s2 + s4)).astype(BF)
                oc(ib).start()
                s7 = _dot((u12 - u22).astype(BF), wb_v[4])
                o_v[ot, 0:DH2] = (et[:, 0:DH2] + ((s1 + s4) + (s7 - s5))).astype(BF)
                oc(it).start()
            return carry

        jax.lax.fori_loop(0, n3, body3, 0)
        for i in range(S // TO):
            oc(i).wait()

    return kernel, n1, n3, nx0


def build(TM1=512, X0=256, TM2=512, SEG=64, TR=512, TO=128, WC=32):
    kernel, n1, n3, nx0 = make_kernel(TM1, X0, TM2, SEG, TR, TO, WC)

    @jax.jit
    def pallas_sequential_preLN__linear_attn_block__mixer_gmlp__prompt_kernel(
            A_x, A_wqkv, A_wo, B_x, B_w_in, B_w_sp, B_b_sp, B_w_out):
        del B_x
        any_spec = pl.BlockSpec(memory_space=pl.ANY)
        return pl.pallas_call(
            kernel,
            out_shape=jax.ShapeDtypeStruct((1, S, D), BF),
            in_specs=[any_spec] * 7,
            out_specs=any_spec,
            scratch_shapes=[
                pltpu.VMEM((S, D), BF),
                pltpu.VMEM((3, D, D), BF),
                pltpu.VMEM((D, D), BF),
                pltpu.VMEM((D, F), BF),
                pltpu.VMEM((S, S), BF),
                pltpu.VMEM((S,), BF),
                pltpu.VMEM((FH, D), BF),
                pltpu.VMEM((S, D), BF),
                pltpu.VMEM((D, D), BF),
                pltpu.VMEM((D, D), BF),
                pltpu.VMEM((D, TM1), BF),
                pltpu.VMEM((D, D), F32),
                pltpu.VMEM((D, 128), F32),
                pltpu.VMEM((D, 128), F32),
                pltpu.VMEM((D, D), BF),
                pltpu.VMEM((S, D), F32),
                pltpu.VMEM((TM2, D), BF),
                pltpu.VMEM((S, FH), BF),
                pltpu.VMEM((7, H2, NH), BF),
                pltpu.VMEM((5, NH, DH2), BF),
                pltpu.VMEM((S, 128), BF),
                pltpu.VMEM((S, 128), F32),
                pltpu.VMEM((S, D), BF),
                pltpu.SemaphoreType.DMA((nx0,)),
                pltpu.SemaphoreType.DMA((n1,)),
                pltpu.SemaphoreType.DMA((7,)),
                pltpu.SemaphoreType.DMA((2 * n3,)),
                pltpu.SemaphoreType.DMA((1,)),
            ],
            compiler_params=pltpu.CompilerParams(vmem_limit_bytes=100 * 2**20),
        )(A_x, A_wqkv, A_wo, B_w_in, B_w_sp, B_b_sp, B_w_out)

    return pallas_sequential_preLN__linear_attn_block__mixer_gmlp__prompt_kernel


pallas_sequential_preLN__linear_attn_block__mixer_gmlp__prompt_kernel = build()
```
